```python
import jax
import jax.numpy as jnp

def _softmax(x, axis=-1):
    return jax.nn.softmax(x, axis=axis)

def _gelu(x):
    return jax.nn.gelu(x, approximate=True)

def _silu(x):
    return jax.nn.silu(x)

def _sigmoid(x):
    return jax.nn.sigmoid(x)

def _layernorm(x, axis=-1, eps=1e-05):
    m = jnp.mean(x, axis=axis, keepdims=True)
    v = jnp.var(x, axis=axis, keepdims=True)
    return (x - m) / jnp.sqrt(v + eps)

def _scatter_add(tgt, idx, src, axis=0):
    return tgt.at[idx].add(src)

def _segment_sum(src, seg, n):
    return jax.ops.segment_sum(src, seg, n)

class _Rng:

    def __init__(self, key):
        self._k = key

    def _next(self):
        self._k, sub = jax.random.split(self._k)
        return sub

    def normal(self, shape):
        return jax.random.normal(self._next(), shape, dtype=jnp.bfloat16)

    def randint(self, lo, hi, shape):
        return jax.random.randint(self._next(), shape, lo, hi, dtype=jnp.int32)

    def uniform(self, shape, lo=0.0, hi=1.0):
        return jax.random.uniform(self._next(), shape, jnp.bfloat16, lo, hi)

    def permutation(self, n):
        return jax.random.permutation(self._next(), n)
kernel_name = 'standalone__conformer_conv_module__speech'

def setup_inputs():
    _rng = _Rng(jax.random.key(int.from_bytes(__import__("os").urandom(4), "little")))
    _w = lambda a: (lambda t: t.astype(jnp.bfloat16) if jnp.issubdtype(t.dtype, jnp.floating) else t)(jnp.asarray(a))
    B, T, D, K = (2, 16000, 256, 31)
    return {'x': _w((lambda *s: _rng.normal(s) * 0.05)(B, T, D)), 'w_pw1': _w((lambda *s: _rng.normal(s) * 0.05)(D, 2 * D)), 'dw': _w((lambda *s: _rng.normal(s) * 0.05)(K, D)), 'w_pw2': _w((lambda *s: _rng.normal(s) * 0.05)(D, D))}

def reference(x, w_pw1, dw, w_pw2):
    B, T, D = x.shape
    K = dw.shape[0]
    h = x @ w_pw1
    a, b = (h[..., :D].copy(), h[..., D:].copy())
    h = a * _sigmoid(b)
    pad = K // 2
    hp = jnp.pad(h, ((0, 0), (pad, pad), (0, 0)))
    out = jnp.zeros_like(h)
    for i in range(K):
        out = out + hp[:, i:i + T, :] * dw[i][None, None, :]
    return _silu(out) @ w_pw2
```

```python
import functools
import jax
import jax.numpy as jnp
import jax.experimental.pallas as pl
import jax.experimental.pallas.tpu as pltpu

D = 256
S = 8
CJ = 80
P = 81
LEV = 3
G = 4
DB = 5
F32 = jnp.float32
BF = jnp.bfloat16


def _leaf_weights(g, lev):
    if lev == 0:
        return [g]
    ge, go = g[0::2], g[1::2]
    gs = [b if a is None else a + b for a, b in zip(ge, go)]
    return _leaf_weights(gs, lev - 1) + _leaf_weights(go, lev - 1) + _leaf_weights(ge, lev - 1)


def _body(x_hbm, w1_ref, dw_ref, w2_ref, o_hbm, xb, ob, h0, h1, y0, y1, wl, cr, w1s, isem, psem, osem, *, L):
    NC = L // CJ
    NT = 32 >> LEV
    hb = (h0, h1)
    yb = (y0, y1)
    NB = 2 * NC // DB

    def in_copy(q):
        b, r = q // (NC // DB), q % (NC // DB)
        s0 = pl.multiple_of(b * S, S)
        r0 = pl.multiple_of(r * (DB * CJ), 16)
        return pltpu.make_async_copy(x_hbm.at[pl.ds(s0, S), pl.ds(r0, DB * CJ)],
                                     xb.at[pl.ds(s0, S), pl.ds(r0 + 16, DB * CJ)], isem.at[q])

    def out_copy(c):
        b, r = c // NC, c % NC
        s0 = pl.multiple_of(b * S, S)
        r0 = pl.multiple_of(r * CJ, 16)
        return pltpu.make_async_copy(ob.at[pl.ds(s0, S), pl.ds(r0, CJ)],
                                     o_hbm.at[pl.ds(s0, S), pl.ds(r0, CJ)], osem)

    pads = []
    for b in range(2):
        pads.append(pltpu.make_async_copy(x_hbm.at[pl.ds(b * S, S - 1), pl.ds(L - 16, 16)],
                                          xb.at[pl.ds(b * S + 1, S - 1), pl.ds(0, 16)], psem.at[2 * b]))
        pads.append(pltpu.make_async_copy(x_hbm.at[pl.ds(b * S + 1, S - 1), pl.ds(0, 16)],
                                          xb.at[pl.ds(b * S, S - 1), pl.ds(L + 16, 16)], psem.at[2 * b + 1]))
    pads[0].start()
    in_copy(0).start()
    for p in pads[1:]:
        p.start()
    for q in range(1, NB):
        in_copy(q).start()
    z16 = jnp.zeros((16, D), BF)
    for b in range(2):
        xb[b * S, 0:16, :] = z16
        xb[b * S + S - 1, L + 16:L + 32, :] = z16

    for l in range(2):
        for t in range(2):
            w1s[l, :, t * 128:(t + 1) * 128] = (w1_ref[:, t * D + l * 128:t * D + (l + 1) * 128].astype(F32) * 0.5).astype(BF)
    dw = dw_ref[...].astype(F32) * 0.5
    live = []
    for l in range(2):
        g = [None] + [jnp.broadcast_to(dw[31 - k:32 - k, l * 128:(l + 1) * 128], (8, 128)) for k in range(1, 32)]
        lw = _leaf_weights(g, LEV)
        live = [[t is not None for t in w] for w in lw]
        for i, w in enumerate(lw):
            for t in range(NT):
                if w[t] is not None:
                    wl[l, i * NT + t] = w[t]

    def mm1(b, r0, n, hbuf):
        s0 = pl.multiple_of(b * S, S)
        for g in range(0, S, G):
            for l in range(2):
                xv = xb[pl.ds(s0 + g, G), pl.ds(r0, n), :].reshape(G * n, D)
                z = jnp.dot(xv, w1s[l], preferred_element_type=F32)
                for s in range(G):
                    a = z[s * n:(s + 1) * n, :128]
                    hbuf[l, (g + s) * P:(g + s) * P + n, :] = a * jnp.tanh(z[s * n:(s + 1) * n, 128:]) + a
                yield

    def conv(hbuf, ybuf, n, prime):
        for l in range(2):
            cnt = [0, 0]

            def carry(new):
                i = cnt[0]
                cnt[0] += 1
                old = jnp.zeros((8, 128), F32) if prime else cr[l, i]
                cr[l, i] = new
                return old

            def fir(x, lev, emit):
                if lev == 0:
                    li = cnt[1]
                    cnt[1] += 1
                    old = [carry(v) for v in x[len(x) - (NT - 1):]]
                    if prime:
                        return
                    xx = old + x
                    w = [wl[l, li * NT + t] if live[li][t] else None for t in range(NT)]
                    for m in range(len(x)):
                        acc = None
                        for t in range(NT):
                            if w[t] is None:
                                continue
                            pr = w[t] * xx[m + NT - 1 - t]
                            acc = pr if acc is None else acc + pr
                        emit(m, acc)
                    yield
                    return
                xe, xo = x[0::2], x[1::2]
                prev = [carry(xo[-1])] + xo[:-1]
                m2 = {}
                yield from fir(xe, lev - 1, m2.__setitem__)
                yield from fir([p - e for p, e in zip(prev, xe)], lev - 1, lambda m, v: emit(2 * m, m2[m] + v))
                yield from fir([o - e for o, e in zip(xo, xe)], lev - 1, lambda m, v: emit(2 * m + 1, m2[m] + v))

            def fin(j, v):
                ybuf[l, pl.ds(j, S, stride=P), :] = v * jnp.tanh(v) + v

            yield from fir([hbuf[l, pl.ds(j, S, stride=P), :] for j in range(n)], LEV, fin)

    def mm2(c, ybuf):
        b, r = c // NC, c % NC
        s0 = pl.multiple_of(b * S, S)
        r0 = pl.multiple_of(r * CJ, 16)
        for g in range(0, S, G):
            yv = jnp.concatenate([
                jnp.concatenate([ybuf[l, s * P:s * P + CJ, :] for l in range(2)], axis=1).astype(BF)
                for s in range(g, g + G)], axis=0)
            o = jnp.dot(yv, w2_ref[...], preferred_element_type=F32).astype(BF)
            for s in range(G):
                ob[s0 + g + s, pl.ds(r0, CJ), :] = o[s * CJ:(s + 1) * CJ]
            yield

    def mm1c(c, hbuf):
        b, r = c // NC, c % NC
        return mm1(b, pl.multiple_of(r * CJ + 32, 16), CJ, hbuf)

    def run(*gens):
        for g in gens:
            for _ in g:
                pass

    def mix(cv, *mms):
        nm = sum(n for _, n in mms)
        nl = 2 * 3 ** LEV
        done = 0
        k = 0
        for g, n in mms:
            for _ in range(n):
                next(g)
                k += 1
                while done < k * nl // nm:
                    next(cv)
                    done += 1
        run(cv)

    def prime(b, hbuf):
        run(mm1(b, 0, 32, hbuf), conv(hbuf, None, 32, True))

    def wait_for(c):
        c = jnp.int32(c)
        nxt = c + 1
        @pl.when(jnp.logical_and(nxt % DB == 0, nxt < 2 * NC))
        def _():
            in_copy(nxt // DB).wait()

    for p in pads:
        p.wait()
    in_copy(0).wait()
    prime(0, h1)
    run(mm1c(0, h0))
    mix(conv(h0, y0, CJ, False), (mm1c(1, h1), 2 * S // G))

    def step(i, par):
        mix(conv(hb[1 - par], yb[1 - par], CJ, False), (mm1c(i, hb[par]), 2 * S // G), (mm2(i - 2, yb[par]), S // G))

    def pair(k, _):
        i = 2 + 2 * k
        wait_for(i)
        wait_for(i + 1)
        @pl.when(i == NC + 1)
        def _():
            prime(1, h0)
        step(i, 0)
        step(i + 1, 1)
        out_copy(i - 2).start()
        out_copy(i - 1).start()
        return 0

    jax.lax.fori_loop(0, NC - 1, pair, 0)
    mix(conv(h1, y1, CJ, False), (mm2(2 * NC - 2, y0), S // G))
    out_copy(2 * NC - 2).start()
    run(mm2(2 * NC - 1, y1))
    out_copy(2 * NC - 1).start()
    pltpu.make_async_copy(ob, o_hbm, osem).wait()


@jax.jit
def pallas_standalone__conformer_conv_module__speech_kernel(x, w_pw1, dw, w_pw2):
    B, T, _ = x.shape
    L = T // S
    NL = 3 ** LEV * (32 >> LEV)
    vm = pl.BlockSpec(memory_space=pltpu.VMEM)
    out = pl.pallas_call(
        functools.partial(_body, L=L),
        in_specs=[pl.BlockSpec(memory_space=pl.ANY), vm, vm, vm],
        out_specs=pl.BlockSpec(memory_space=pl.ANY),
        out_shape=jax.ShapeDtypeStruct((B * S, L, D), x.dtype),
        scratch_shapes=[
            pltpu.VMEM((B * S, L + 32, D), BF), pltpu.VMEM((B * S, L, D), BF),
            *[pltpu.VMEM((2, S * P + 8, 128), F32) for _ in range(4)],
            pltpu.VMEM((2, NL, 8, 128), F32), pltpu.VMEM((2, NL, 8, 128), F32),
            pltpu.VMEM((2, D, D), BF),
            pltpu.SemaphoreType.DMA((2 * L // CJ // DB,)), pltpu.SemaphoreType.DMA((4,)), pltpu.SemaphoreType.DMA(()),
        ],
        compiler_params=pltpu.CompilerParams(vmem_limit_bytes=64 << 20),
    )(x.reshape(B * S, L, D), w_pw1, dw, w_pw2)
    return out.reshape(B, T, D)
```
